```python
import os as _os
_os.environ.setdefault("JAX_PLATFORMS", "cpu")
import jax
import jax.numpy as jnp

def _softmax(x, axis=-1):
    return jax.nn.softmax(x, axis=axis)
def _gelu(x):
    return jax.nn.gelu(x, approximate=True)
def _silu(x):
    return jax.nn.silu(x)
def _sigmoid(x):
    return jax.nn.sigmoid(x)
def _layernorm(x, axis=-1, eps=1e-5):
    m = jnp.mean(x, axis=axis, keepdims=True)
    v = jnp.var(x, axis=axis, keepdims=True)
    return (x - m) / jnp.sqrt(v + eps)
def _scatter_add(tgt, idx, src, axis=0):
    return tgt.at[idx].add(src)
def _segment_sum(src, seg, n):
    return jax.ops.segment_sum(src, seg, n)
class _Rng:
    def __init__(self, key):
        self._k = key
    def _next(self):
        self._k, sub = jax.random.split(self._k)
        return sub
    def normal(self, shape):
        return jax.random.normal(self._next(), shape, dtype=jnp.bfloat16)
    def randint(self, lo, hi, shape):
        return jax.random.randint(self._next(), shape, lo, hi, dtype=jnp.int32)
    def uniform(self, shape, lo=0.0, hi=1.0):
        return jax.random.uniform(self._next(), shape, jnp.bfloat16, lo, hi)
    def permutation(self, n):
        return jax.random.permutation(self._next(), n)


kernel_name = 'standalone__gqa_block_cached__near_ridge'

def setup_inputs():
    _rng = _Rng(jax.random.key(int.from_bytes(__import__("os").urandom(4), "little")))
    _w = (lambda a: (lambda t: t.astype(jnp.bfloat16) if jnp.issubdtype(t.dtype, jnp.floating) else t)(jnp.asarray(a)))
    B, Sq, D = 8, 96, 448
    Hq, Hkv, Sk, Dh = 16, 8, 2048, 256
    assert Hq % Hkv == 0, (Hq, Hkv)
    return {
        "x": _w((lambda *s: _rng.normal(s) * 0.8)(B, Sq, D)),
        "k_cache": _w((lambda *s: _rng.normal(s) * 0.8)(B, Hkv, Sk, Dh)),
        "v_cache": _w((lambda *s: _rng.normal(s) * 0.05)(B, Hkv, Sk, Dh)),
        "wq": _w((lambda *s: _rng.normal(s) * 0.8)(D, Hq * Dh) * (D ** -0.5)),
        "wo": _w((lambda *s: _rng.normal(s) * 0.05)(Hq * Dh, D) * ((Hq * Dh) ** -0.5)),
    }

def reference(x, k_cache, v_cache, wq, wo):
    B, Sq, D = x.shape
    Hq, Dh = 16, 256
    Hkv = k_cache.shape[1]
    rep = Hq // Hkv
    q = (lambda x, *d: x.transpose(*d))((x @ wq).reshape(B, Sq, Hq, Dh), 0, 2, 1, 3)
    k = jnp.repeat(k_cache, rep, axis=1)
    v = jnp.repeat(v_cache, rep, axis=1)
    scores = jnp.einsum("bhqd,bhkd->bhqk", q, k) * (Dh ** -0.5)
    p = _softmax(scores, axis=-1)
    o = jnp.einsum("bhqk,bhkd->bhqd", p, v)
    return (lambda x, *d: x.transpose(*d))(o, 0, 2, 1, 3).reshape(B, Sq, Hq * Dh) @ wo
```

```python
import jax
import jax.numpy as jnp
from jax import lax
from jax.experimental import pallas as pl
from jax.experimental.pallas import tpu as pltpu

B, SQ, D = 8, 96, 448
HKV, SK, DH = 8, 2048, 256
REP = 2
M = REP * SQ
HW = REP * DH
NS = B * HKV
NB = 4
CH = 256
NT = (((1,), (1,)), ((), ()))
F32, BF16 = jnp.float32, jnp.bfloat16


def _kernel(x_hbm, k_hbm, v_hbm, wq_hbm, wot_hbm, o_hbm,
            xb, wqb, wob, kb, vb, acc, ob, qbuf, sbuf, mbuf,
            sem_k, sem_v, sem_w, sem_x, sem_o):
    bi = lambda i: i & (B - 1)
    hi = lambda i: i >> 3
    sl = lambda i: i & (NB - 1)

    def kcp(i):
        return pltpu.make_async_copy(k_hbm.at[bi(i), hi(i)], kb.at[sl(i)], sem_k.at[sl(i)])

    def vcp(i):
        return pltpu.make_async_copy(v_hbm.at[bi(i), hi(i)], vb.at[sl(i)], sem_v.at[sl(i)])

    def wqcp(h):
        return pltpu.make_async_copy(
            wq_hbm.at[:, pl.ds(pl.multiple_of(h * HW, HW), HW)], wqb.at[h], sem_w.at[h])

    def wocp(h):
        return pltpu.make_async_copy(
            wot_hbm.at[:, pl.ds(pl.multiple_of(h * HW, HW), HW)], wob.at[h], sem_w.at[HKV + h])

    def ocp(b):
        return pltpu.make_async_copy(ob.at[b], o_hbm.at[b], sem_o.at[b])

    xcp = pltpu.make_async_copy(x_hbm, xb, sem_x)

    def qproj(i):
        q = jnp.dot(xb[bi(i)], wqb[hi(i)], preferred_element_type=F32) * (DH ** -0.5)
        q = q.astype(BF16)
        qbuf[i & 1, 0:SQ, :] = q[:, :DH]
        qbuf[i & 1, SQ:M, :] = q[:, DH:]

    def qk(i):
        q2 = qbuf[i & 1]
        mm = None
        for c in range(SK // CH):
            s = lax.dot_general(q2, kb[sl(i), c * CH:(c + 1) * CH, :], NT, preferred_element_type=F32)
            sbuf[i & 1, :, c * CH:(c + 1) * CH] = s
            for t in range(CH // 128):
                st = s[:, t * 128:(t + 1) * 128]
                mm = st if mm is None else jnp.maximum(mm, st)
        m = jnp.max(mm, axis=-1, keepdims=True)
        mbuf[i & 1] = jnp.broadcast_to(m, (M, 128))

    def smpv(i):
        m = mbuf[i & 1]
        o = ll = None
        for c in range(SK // CH):
            ps = []
            for t in range(CH // 128):
                c0 = c * CH + t * 128
                p = jnp.exp(sbuf[i & 1, :, c0:c0 + 128] - m)
                ll = p if ll is None else ll + p
                ps.append(p.astype(BF16))
            oc = jnp.dot(jnp.concatenate(ps, axis=1), vb[sl(i), c * CH:(c + 1) * CH, :],
                         preferred_element_type=F32)
            o = oc if o is None else o + oc
        l = jnp.sum(ll, axis=-1, keepdims=True)
        o = (o * (1.0 / l)).astype(BF16)
        return jnp.concatenate([o[:SQ], o[SQ:]], axis=1)

    def oproj(i, o2):
        return lax.dot_general(o2, wob[hi(i)], NT, preferred_element_type=F32)

    wqcp(0).start()
    xcp.start()
    kcp(0).start()
    wocp(0).start()
    for j in range(NB - 1):
        vcp(j).start()
        kcp(j + 1).start()
    acc[...] = jnp.zeros_like(acc)
    xcp.wait()
    wqcp(0).wait()
    qproj(0)
    qproj(1)
    kcp(0).wait()
    qk(0)

    def body(i, carry):
        h, b = hi(i), bi(i)

        @pl.when(i + NB < NS)
        def _():
            kcp(i + NB).start()

        @pl.when(i + NB - 1 < NS)
        def _():
            vcp(i + NB - 1).start()

        @pl.when(jnp.logical_and(b == 0, h + 1 < HKV))
        def _():
            wqcp(h + 1).start()
            wocp(h + 1).start()

        @pl.when(jnp.logical_and(b == B - 2, h + 1 < HKV))
        def _():
            wqcp(h + 1).wait()

        @pl.when(b == 0)
        def _():
            wocp(h).wait()

        kcp(i + 1).wait()
        vcp(i).wait()
        qproj(i + 2)
        o2 = smpv(i)
        qk(i + 1)
        acc[b] += oproj(i, o2)
        return carry

    lax.fori_loop(0, NS - 2, body, 0)

    i = NS - 2
    kcp(i + 1).wait()
    vcp(i).wait()
    o2 = smpv(i)
    qk(i + 1)
    ob[B - 2] = (acc[B - 2] + oproj(i, o2)).astype(BF16)
    ocp(B - 2).start()
    for b in range(B - 2):
        ob[b] = acc[b].astype(BF16)
        ocp(b).start()
    i = NS - 1
    vcp(i).wait()
    o2 = smpv(i)
    ob[B - 1] = (acc[B - 1] + oproj(i, o2)).astype(BF16)
    ocp(B - 1).start()
    for b in range(B):
        ocp(b).wait()


@jax.jit
def pallas_standalone__gqa_block_cached__near_ridge_kernel(x, k_cache, v_cache, wq, wo):
    hbm = pl.BlockSpec(memory_space=pltpu.HBM)
    return pl.pallas_call(
        _kernel,
        in_specs=[hbm] * 5,
        out_specs=hbm,
        out_shape=jax.ShapeDtypeStruct((B, SQ, D), BF16),
        scratch_shapes=[
            pltpu.VMEM((B, SQ, D), BF16),
            pltpu.VMEM((HKV, D, HW), BF16),
            pltpu.VMEM((HKV, D, HW), BF16),
            pltpu.VMEM((NB, SK, DH), BF16),
            pltpu.VMEM((NB, SK, DH), BF16),
            pltpu.VMEM((B, SQ, D), F32),
            pltpu.VMEM((B, SQ, D), BF16),
            pltpu.VMEM((2, M, DH), BF16),
            pltpu.VMEM((2, M, SK), F32),
            pltpu.VMEM((2, M, 128), F32),
            pltpu.SemaphoreType.DMA((NB,)),
            pltpu.SemaphoreType.DMA((NB,)),
            pltpu.SemaphoreType.DMA((2 * HKV,)),
            pltpu.SemaphoreType.DMA(()),
            pltpu.SemaphoreType.DMA((B,)),
        ],
        compiler_params=pltpu.CompilerParams(vmem_limit_bytes=64 * 1024 * 1024),
    )(x, k_cache, v_cache, wq, wo.T)
```

```python
import jax
import jax.numpy as jnp
from jax import lax
from jax.experimental import pallas as pl
from jax.experimental.pallas import tpu as pltpu

B, SQ, D = 8, 96, 448
HKV, SK, DH = 8, 2048, 256
REP = 2
M = REP * SQ
HW = REP * DH
NS = B * HKV
NB = 4
QA = 4
CH = 256
NT = (((1,), (1,)), ((), ()))
F32, BF16 = jnp.float32, jnp.bfloat16


def _kernel(x_hbm, k_hbm, v_hbm, wq_hbm, wot_hbm, o_hbm,
            xb, wqb, wob, kb, vb, acc, ob, qbuf, sbuf, mbuf,
            sem_k, sem_v, sem_w, sem_x, sem_o):
    bi = lambda i: i & (B - 1)
    hi = lambda i: i >> 3
    sl = lambda i: i & (NB - 1)

    def kcp(i):
        return pltpu.make_async_copy(k_hbm.at[bi(i), hi(i)], kb.at[sl(i)], sem_k.at[sl(i)])

    def vcp(i):
        return pltpu.make_async_copy(v_hbm.at[bi(i), hi(i)], vb.at[sl(i)], sem_v.at[sl(i)])

    def wqcp(h):
        return pltpu.make_async_copy(
            wq_hbm.at[:, pl.ds(pl.multiple_of(h * HW, HW), HW)], wqb.at[h], sem_w.at[h])

    def wocp(h):
        return pltpu.make_async_copy(
            wot_hbm.at[:, pl.ds(pl.multiple_of(h * HW, HW), HW)], wob.at[h], sem_w.at[HKV + h])

    def ocp(b):
        return pltpu.make_async_copy(ob.at[b], o_hbm.at[b], sem_o.at[b])

    xcp = pltpu.make_async_copy(x_hbm, xb, sem_x)

    def qproj(i):
        q = jnp.dot(xb[bi(i)], wqb[hi(i)], preferred_element_type=F32) * (DH ** -0.5)
        q = q.astype(BF16)
        qbuf[i & (2 * QA - 1), 0:SQ, :] = q[:, :DH]
        qbuf[i & (2 * QA - 1), SQ:M, :] = q[:, DH:]

    def qk(i):
        q2 = qbuf[i & (2 * QA - 1)]
        mm = None
        for c in range(SK // CH):
            s = lax.dot_general(q2, kb[sl(i), c * CH:(c + 1) * CH, :], NT, preferred_element_type=F32)
            sbuf[i & 1, :, c * CH:(c + 1) * CH] = s
            for t in range(CH // 128):
                st = s[:, t * 128:(t + 1) * 128]
                mm = st if mm is None else jnp.maximum(mm, st)
        m = jnp.max(mm, axis=-1, keepdims=True)
        mbuf[i & 1] = jnp.broadcast_to(m, (M, 128))

    def smpv(i):
        m = mbuf[i & 1]
        o = ll = None
        for c in range(SK // CH):
            ps = []
            for t in range(CH // 128):
                c0 = c * CH + t * 128
                p = jnp.exp(sbuf[i & 1, :, c0:c0 + 128] - m)
                ll = p if ll is None else ll + p
                ps.append(p.astype(BF16))
            oc = jnp.dot(jnp.concatenate(ps, axis=1), vb[sl(i), c * CH:(c + 1) * CH, :],
                         preferred_element_type=F32)
            o = oc if o is None else o + oc
        l = jnp.sum(ll, axis=-1, keepdims=True)
        o = (o * (1.0 / l)).astype(BF16)
        return jnp.concatenate([o[:SQ], o[SQ:]], axis=1)

    def oproj(i, o2):
        return lax.dot_general(o2, wob[hi(i)], NT, preferred_element_type=F32)

    wqcp(0).start()
    xcp.start()
    kcp(0).start()
    wocp(0).start()
    for j in range(NB - 1):
        vcp(j).start()
        kcp(j + 1).start()
    acc[...] = jnp.zeros_like(acc)
    xcp.wait()
    wqcp(0).wait()
    for j in range(QA):
        qproj(j)
    kcp(0).wait()
    qk(0)

    def body(i, carry):
        h, b = hi(i), bi(i)

        vcp(i + NB - 1).start()
        kcp(i + NB).start()

        @pl.when(jnp.logical_and(b == 0, h + 1 < HKV))
        def _():
            wqcp(h + 1).start()
            wocp(h + 1).start()

        @pl.when(jnp.logical_and(b == B - QA, h + 1 < HKV))
        def _():
            wqcp(h + 1).wait()

        @pl.when(b == 0)
        def _():
            wocp(h).wait()

        kcp(i + 1).wait()
        vcp(i).wait()
        qproj(i + QA)
        o2 = smpv(i)
        qk(i + 1)
        acc[b] += oproj(i, o2)
        return carry

    lax.fori_loop(0, NS - QA, body, 0)

    vcp(NS - 1).start()

    def tail(i, carry):
        vcp(i).wait()
        o2 = smpv(i)
        kcp(i + 1).wait()
        qk(i + 1)
        acc[bi(i)] += oproj(i, o2)
        return carry

    lax.fori_loop(NS - QA, NS - 1, tail, 0)
    for b in range(B - 1):
        ob[b] = acc[b].astype(BF16)
        ocp(b).start()
    i = NS - 1
    vcp(i).wait()
    o2 = smpv(i)
    ob[B - 1] = (acc[B - 1] + oproj(i, o2)).astype(BF16)
    ocp(B - 1).start()
    for b in range(B):
        ocp(b).wait()


@jax.jit
def pallas_standalone__gqa_block_cached__near_ridge_kernel(x, k_cache, v_cache, wq, wo):
    hbm = pl.BlockSpec(memory_space=pltpu.HBM)
    return pl.pallas_call(
        _kernel,
        in_specs=[hbm] * 5,
        out_specs=hbm,
        out_shape=jax.ShapeDtypeStruct((B, SQ, D), BF16),
        scratch_shapes=[
            pltpu.VMEM((B, SQ, D), BF16),
            pltpu.VMEM((HKV, D, HW), BF16),
            pltpu.VMEM((HKV, D, HW), BF16),
            pltpu.VMEM((NB, SK, DH), BF16),
            pltpu.VMEM((NB, SK, DH), BF16),
            pltpu.VMEM((B, SQ, D), F32),
            pltpu.VMEM((B, SQ, D), BF16),
            pltpu.VMEM((2 * QA, M, DH), BF16),
            pltpu.VMEM((2, M, SK), F32),
            pltpu.VMEM((2, M, 128), F32),
            pltpu.SemaphoreType.DMA((NB,)),
            pltpu.SemaphoreType.DMA((NB,)),
            pltpu.SemaphoreType.DMA((2 * HKV,)),
            pltpu.SemaphoreType.DMA(()),
            pltpu.SemaphoreType.DMA((B,)),
        ],
        compiler_params=pltpu.CompilerParams(vmem_limit_bytes=64 * 1024 * 1024),
    )(x, k_cache, v_cache, wq, wo.T)
```
